```python
import jax
import jax.numpy as jnp

def _softmax(x, axis=-1):
    return jax.nn.softmax(x, axis=axis)
def _gelu(x):
    return jax.nn.gelu(x, approximate=True)
def _silu(x):
    return jax.nn.silu(x)
def _sigmoid(x):
    return jax.nn.sigmoid(x)
def _layernorm(x, axis=-1, eps=1e-5):
    m = jnp.mean(x, axis=axis, keepdims=True)
    v = jnp.var(x, axis=axis, keepdims=True)
    return (x - m) / jnp.sqrt(v + eps)
def _scatter_add(tgt, idx, src, axis=0):
    return tgt.at[idx].add(src)
def _segment_sum(src, seg, n):
    return jax.ops.segment_sum(src, seg, n)
class _Rng:
    def __init__(self, key):
        self._k = key
    def _next(self):
        self._k, sub = jax.random.split(self._k)
        return sub
    def normal(self, shape):
        return jax.random.normal(self._next(), shape, dtype=jnp.bfloat16)
    def randint(self, lo, hi, shape):
        return jax.random.randint(self._next(), shape, lo, hi, dtype=jnp.int32)
    def uniform(self, shape, lo=0.0, hi=1.0):
        return jax.random.uniform(self._next(), shape, jnp.bfloat16, lo, hi)
    def permutation(self, n):
        return jax.random.permutation(self._next(), n)


kernel_name = 'gated_mix__sliding_local_dilated__compressed_kv_cla__prompt'

def setup_inputs():
    _rng = _Rng(jax.random.key(int.from_bytes(__import__("os").urandom(4), "little")))
    _w = (lambda a: (lambda t: t.astype(jnp.bfloat16) if jnp.issubdtype(t.dtype, jnp.floating) else t)(jnp.asarray(a)))
    def _A_setup():
        B, S, D = 1, 2048, 576
        return {
            "x": _w((lambda *s: _rng.normal(s) * 0.05)(B, S, D)),
            "wqkv": _w((lambda *s: _rng.normal(s) * 0.05)(D, 3 * D)),
            "wo": _w((lambda *s: _rng.normal(s) * 0.05)(D, D)),
        }
    _A_in = _A_setup()

    def _B_setup():
        B, H, Sq, Sk, D, M = 1, 32, 2048, 2048, 128, 576
        Dc = 4 * D
        return {
            "x": _w((lambda *s: _rng.normal(s) * 0.05)(B, Sq, M)),
            "c_kv": _w((lambda *s: _rng.normal(s) * 0.05)(B, Sk, Dc)),
            "w_q": _w((lambda *s: _rng.normal(s) * 0.05)(M, H, D) * (M ** -0.5)),
            "w_uk": _w((lambda *s: _rng.normal(s) * 0.05)(Dc, H, D) * (Dc ** -0.5)),
            "w_uv": _w((lambda *s: _rng.normal(s) * 0.05)(Dc, H, D) * (Dc ** -0.5)),
            "w_o": _w((lambda *s: _rng.normal(s) * 0.05)(H, D, M) * ((H * D) ** -0.5)),
        }
    _B_in = _B_setup()

    return {
        "A_x": _A_in["x"],
        "A_wqkv": _A_in["wqkv"],
        "A_wo": _A_in["wo"],
        "B_x": _B_in["x"],
        "B_c_kv": _B_in["c_kv"],
        "B_w_q": _B_in["w_q"],
        "B_w_uk": _B_in["w_uk"],
        "B_w_uv": _B_in["w_uv"],
        "B_w_o": _B_in["w_o"],
        "gate_w": _w((lambda *s: _rng.normal(s) * 0.05)(576)),
    }

def reference(A_x, A_wqkv, A_wo, B_x, B_c_kv, B_w_q, B_w_uk, B_w_uv, B_w_o, gate_w):
    def _A_ref(x, wqkv, wo):
        B, S, D = x.shape
        H = 32; Dh = D // H
        W, dil = 8, 2
        qkv = (lambda x, *d: x.transpose(*d))((x @ wqkv).reshape(B, S, 3, H, Dh), 2, 0, 3, 1, 4)
        q, k, v = qkv[0], qkv[1], qkv[2]
        scale = Dh ** -0.5
        pos = jnp.arange(S)
        off = jnp.arange(W) * dil
        idx = pos[:, None] - off[None, :]
        mask = idx >= 0
        idx_c = jnp.where(mask, idx, 0).reshape(-1)
        kg = k[:, :, idx_c, :].reshape(B, H, S, W, Dh)
        vg = v[:, :, idx_c, :].reshape(B, H, S, W, Dh)
        logits = jnp.einsum("bhsd,bhswd->bhsw", q, kg) * scale
        logits = jnp.where(mask[None, None, :, :], logits, -1e9)
        attn = _softmax(logits, axis=-1)
        o = jnp.einsum("bhsw,bhswd->bhsd", attn, vg)
        return (lambda x, *d: x.transpose(*d))(o, 0, 2, 1, 3).reshape(B, S, D) @ wo

    def _B_ref(x, c_kv, w_q, w_uk, w_uv, w_o):
        B, Sq, M = x.shape[0], x.shape[1], x.shape[2]
        Sk = c_kv.shape[1]
        H, D = w_q.shape[1], w_q.shape[2]
        q = jnp.einsum("bqm,mhd->bhqd", x, w_q)
        k = jnp.einsum("bkc,chd->bhkd", c_kv, w_uk)
        v = jnp.einsum("bkc,chd->bhkd", c_kv, w_uv)
        scores = jnp.einsum("bhqd,bhkd->bhqk", q, k) * (D ** -0.5)
        off = Sk - Sq
        qi = jnp.arange(Sq)[:, None]
        kj = jnp.arange(Sk)[None, :]
        cmask = kj <= (qi + off)
        scores = jnp.where(cmask[None, None], scores, -1e9)
        p = _softmax(scores, axis=-1)
        ctx = jnp.einsum("bhqk,bhkd->bhqd", p, v)
        return jnp.einsum("bhqd,hdm->bqm", ctx, w_o)

    x = A_x
    g = _sigmoid((x * gate_w).sum(-1, keepdims=True))
    a = _A_ref(x, A_wqkv, A_wo)
    b = _B_ref(x, B_c_kv, B_w_q, B_w_uk, B_w_uv, B_w_o)
    return g * a + (1 - g) * b
```

```python
import numpy as np
import jax
import jax.numpy as jnp
import jax.experimental.pallas as pl
import jax.experimental.pallas.tpu as pltpu

S = 2048
M = 576
H = 32
DH = 18
D = 128
DC = 512
WIN, DIL = 8, 2
BQ = 256
LOG2E = 1.4426950408889634
BF = jnp.bfloat16
F32 = jnp.float32
NT = (((1,), (1,)), ((), ()))


def _pair(w_ref, j):
    w = w_ref.bitcast(jnp.uint32)[:, j, :]
    lo = pltpu.bitcast(w << 16, F32).astype(BF)
    hi = pltpu.bitcast(w & np.uint32(0xFFFF0000), F32).astype(BF)
    return jnp.concatenate([lo, hi], axis=1)


def _kernel(x_ref, wqkv_ref, woa_ref, c_ref, wq_ref, wk_ref, wv_ref, wob_ref, g_ref,
            o_ref, q_s, k_s, v_s, ctx_s, ka_s, va_s, oa_s):
    PAD = 16
    ind = (jax.lax.broadcasted_iota(jnp.int32, (M, 128), 0) // DH
           == jax.lax.broadcasted_iota(jnp.int32, (M, 128), 1)).astype(BF)
    indt = (jax.lax.broadcasted_iota(jnp.int32, (128, M), 1) // DH
            == jax.lax.broadcasted_iota(jnp.int32, (128, M), 0)).astype(BF)
    ka_s[0:PAD, :] = jnp.zeros((PAD, M), F32)
    va_s[0:PAD, :] = jnp.zeros((PAD, M), F32)
    RA = 256

    def a_body(i, _):
        r0 = pl.multiple_of(i * RA, RA)
        x = x_ref[pl.ds(r0, RA), :]
        q = jnp.dot(x, wqkv_ref[:, 0:M], preferred_element_type=F32) * (DH ** -0.5 * LOG2E)
        ka_s[PAD:PAD + RA, :] = jnp.dot(x, wqkv_ref[:, M:2 * M], preferred_element_type=F32)
        va_s[PAD:PAD + RA, :] = jnp.dot(x, wqkv_ref[:, 2 * M:3 * M], preferred_element_type=F32)
        pos = r0 + jax.lax.broadcasted_iota(jnp.int32, (RA, 128), 0)
        lg = []
        for w in range(WIN):
            kk = ka_s[PAD - w * DIL:PAD - w * DIL + RA, :]
            l = jnp.dot((q * kk).astype(BF), ind, preferred_element_type=F32)
            lg.append(jnp.where(pos >= w * DIL, l, -1e9) if w else l)
        m = lg[0]
        for l in lg[1:]:
            m = jnp.maximum(m, l)
        p = [jnp.exp2(l - m) for l in lg]
        den = p[0]
        for t in p[1:]:
            den = den + t
        inv = 1.0 / den
        o = None
        for w in range(WIN):
            pw = jnp.dot((p[w] * inv).astype(BF), indt, preferred_element_type=F32)
            t = pw * va_s[PAD - w * DIL:PAD - w * DIL + RA, :]
            o = t if o is None else o + t
        oa_s[pl.ds(r0, RA), :] = o.astype(BF)
        ka_s[0:PAD, :] = ka_s[RA:RA + PAD, :]
        va_s[0:PAD, :] = va_s[RA:RA + PAD, :]
        return 0

    jax.lax.fori_loop(0, S // RA, a_body, 0)

    tri = (jax.lax.broadcasted_iota(jnp.int32, (BQ, BQ), 1)
           <= jax.lax.broadcasted_iota(jnp.int32, (BQ, BQ), 0))

    def b_body(j, _):
        q_s[...] = (jnp.dot(x_ref[...], _pair(wq_ref, j), preferred_element_type=F32)
                    * (D ** -0.5 * LOG2E)).astype(BF)
        k_s[...] = jnp.dot(c_ref[...], _pair(wk_ref, j), preferred_element_type=F32).astype(BF)
        v_s[...] = jnp.dot(c_ref[...], _pair(wv_ref, j), preferred_element_type=F32).astype(BF)
        for hh in range(2):
            c0 = hh * D
            for i in range(S // BQ):
                r0, L = i * BQ, (i + 1) * BQ
                q = q_s[r0:L, c0:c0 + D]
                sd = jax.lax.dot_general(q, k_s[r0:L, c0:c0 + D], NT, preferred_element_type=F32)
                sd = jnp.where(tri, sd, -1e9)
                m = jnp.max(sd, axis=1, keepdims=True)
                if i:
                    sf = jax.lax.dot_general(q, k_s[0:r0, c0:c0 + D], NT, preferred_element_type=F32)
                    m = jnp.maximum(m, jnp.max(sf, axis=1, keepdims=True))
                pd = jnp.exp2(sd - m)
                l = jnp.sum(pd, axis=1, keepdims=True)
                o = jnp.dot(pd.astype(BF), v_s[r0:L, c0:c0 + D], preferred_element_type=F32)
                if i:
                    pf = jnp.exp2(sf - m)
                    l = l + jnp.sum(pf, axis=1, keepdims=True)
                    o = o + jnp.dot(pf.astype(BF), v_s[0:r0, c0:c0 + D], preferred_element_type=F32)
                ctx_s[r0:L, pl.ds(pl.multiple_of(j * 2 * D + c0, D), D)] = (o * (1.0 / l)).astype(BF)
        return 0

    jax.lax.fori_loop(0, H // 2, b_body, 0)

    RO = 256

    def o_body(i, _):
        r0 = pl.multiple_of(i * RO, RO)
        x = x_ref[pl.ds(r0, RO), :].astype(F32)
        g = jax.nn.sigmoid(jnp.sum(x * g_ref[...].astype(F32), axis=1, keepdims=True))
        a = jnp.dot(oa_s[pl.ds(r0, RO), :], woa_ref[...], preferred_element_type=F32)
        b = jnp.dot(ctx_s[pl.ds(r0, RO), :], wob_ref[...], preferred_element_type=F32)
        o_ref[pl.ds(r0, RO), :] = (g * a + (1.0 - g) * b).astype(o_ref.dtype)
        return 0

    jax.lax.fori_loop(0, S // RO, o_body, 0)


@jax.jit
def pallas_gated_mix__sliding_local_dilated__compressed_kv_cla__prompt_kernel(
    A_x, A_wqkv, A_wo, B_x, B_c_kv, B_w_q, B_w_uk, B_w_uv, B_w_o, gate_w,
):
    del B_x
    out = pl.pallas_call(
        _kernel,
        out_shape=jax.ShapeDtypeStruct((S, M), A_x.dtype),
        scratch_shapes=[
            pltpu.VMEM((S, 2 * D), BF), pltpu.VMEM((S, 2 * D), BF), pltpu.VMEM((S, 2 * D), BF),
            pltpu.VMEM((S, H * D), BF),
            pltpu.VMEM((256 + 16, M), F32), pltpu.VMEM((256 + 16, M), F32),
            pltpu.VMEM((S, M), BF),
        ],
        compiler_params=pltpu.CompilerParams(vmem_limit_bytes=110 * 1024 * 1024),
    )(A_x.reshape(S, M), A_wqkv, A_wo, B_c_kv.reshape(S, DC), B_w_q, B_w_uk, B_w_uv,
      B_w_o.reshape(H * D, M), gate_w.reshape(1, M))
    return out.reshape(1, S, M)
```

```python
import numpy as np
import jax
import jax.numpy as jnp
import jax.experimental.pallas as pl
import jax.experimental.pallas.tpu as pltpu

S = 2048
M = 576
H = 32
DH = 18
D = 128
DC = 512
WIN, DIL = 8, 2
BQ = 256
CA = 256
NQ = 3 * M + 16
LOG2E = 1.4426950408889634
BF = jnp.bfloat16
F32 = jnp.float32
NT = (((1,), (1,)), ((), ()))


def _split_heads(src, dst, i, kb):
    blk = src.bitcast(jnp.uint32).at[pl.ds(pl.multiple_of(i * (kb * H // 2), 8), kb * H // 2)]
    r0 = pl.multiple_of(i * kb, kb)
    for j in range(H // 2):
        w = blk[pl.ds(j, kb, stride=H // 2), :]
        dst[2 * j, pl.ds(r0, kb), :] = pltpu.bitcast(w << 16, F32).astype(BF)
        dst[2 * j + 1, pl.ds(r0, kb), :] = pltpu.bitcast(w & np.uint32(0xFFFF0000), F32).astype(BF)


def _pair(w_ref, j):
    return jnp.concatenate([w_ref[2 * j], w_ref[2 * j + 1]], axis=1)


def _kernel(xt_h, wqkv_h, woa_h, c_h, wq_h, wk_h, wv_h, wob_h, g_ref, o_ref,
            xt, wqkv, woa, c, wq, wk, wv, wob,
            x_s, wt_s, woat_s, qkv_s, oa_s, q_s, k_s, v_s, ctx_s, wq_s, wk_s, wv_s, sems):
    srcs = (wqkv_h, xt_h, c_h, wq_h, wk_h, wv_h, woa_h, wob_h)
    dsts = (wqkv, xt, c, wq, wk, wv, woa, wob)
    cps = [pltpu.make_async_copy(a, b, sems.at[i]) for i, (a, b) in enumerate(zip(srcs, dsts))]
    for cp in cps:
        cp.start()

    cps[0].wait()
    for t in range(3):
        wt_s[t * M:(t + 1) * M, :] = wqkv[:, t * M:(t + 1) * M].astype(F32).T.astype(BF)
    wt_s[3 * M:NQ, :] = jnp.broadcast_to(g_ref[...], (16, M))
    cps[1].wait()

    def p1(i, _):
        c0 = pl.multiple_of(i * CA, CA)
        xc = xt[:, pl.ds(c0, CA)]
        r = jnp.dot(wt_s[...], xc, preferred_element_type=F32)
        for u in range(CA // 128):
            qkv_s[i * (CA // 128) + u] = r[:, u * 128:(u + 1) * 128]
        x_s[pl.ds(c0, CA), :] = xc.astype(F32).T.astype(BF)
        return 0

    jax.lax.fori_loop(0, S // CA, p1, 0)

    for i in (2, 3, 4, 5):
        cps[i].wait()

    def split(i, _):
        _split_heads(wq, wq_s, i, M // 4)
        _split_heads(wk, wk_s, i, DC // 4)
        _split_heads(wv, wv_s, i, DC // 4)
        return 0

    jax.lax.fori_loop(0, 4, split, 0)
    tri = (jax.lax.broadcasted_iota(jnp.int32, (BQ, BQ), 1)
           <= jax.lax.broadcasted_iota(jnp.int32, (BQ, BQ), 0))

    def b_body(j, _):
        q2 = (jnp.dot(x_s[...], _pair(wq_s, j), preferred_element_type=F32)
              * (D ** -0.5 * LOG2E)).astype(BF)
        k2 = jnp.dot(c[...], _pair(wk_s, j), preferred_element_type=F32).astype(BF)
        v2 = jnp.dot(c[...], _pair(wv_s, j), preferred_element_type=F32).astype(BF)
        for hh in range(2):
            q_s[hh] = q2[:, hh * D:(hh + 1) * D]
            k_s[hh] = k2[:, hh * D:(hh + 1) * D]
            v_s[hh] = v2[:, hh * D:(hh + 1) * D]
        for hh in range(2):
            for i in range(S // BQ):
                r0, L = i * BQ, (i + 1) * BQ
                q = q_s[hh, r0:L, :]
                sd = jax.lax.dot_general(q, k_s[hh, r0:L, :], NT, preferred_element_type=F32)
                sd = jnp.where(tri, sd, -1e9)
                m = jnp.max(sd, axis=1, keepdims=True)
                if i:
                    sf = jax.lax.dot_general(q, k_s[hh, 0:r0, :], NT, preferred_element_type=F32)
                    m = jnp.maximum(m, jnp.max(sf, axis=1, keepdims=True))
                pd = jnp.exp2(sd - m)
                l = jnp.sum(pd, axis=1, keepdims=True)
                o = jnp.dot(pd.astype(BF), v_s[hh, r0:L, :], preferred_element_type=F32)
                if i:
                    pf = jnp.exp2(sf - m)
                    l = l + jnp.sum(pf, axis=1, keepdims=True)
                    o = o + jnp.dot(pf.astype(BF), v_s[hh, 0:r0, :], preferred_element_type=F32)
                ctx_s[2 * j + hh, r0:L, :] = (o * (1.0 / l)).astype(BF)
        return 0

    jax.lax.fori_loop(0, H // 2, b_body, 0)

    cps[6].wait()
    woat_s[...] = woa[...].astype(F32).T.astype(BF)
    cps[7].wait()

    def p3(i, _):
        c0 = pl.multiple_of(i * CA, CA)
        for u in range(CA // 128):
            t = i * (CA // 128) + u
            tp = jnp.maximum(t - 1, 0)
            pos = t * 128 + jax.lax.broadcasted_iota(jnp.int32, (H, 128), 1)

            def rows(tt, base):
                return qkv_s[tt, pl.ds(base, H, stride=DH), :]

            def shifted(base):
                e = jnp.concatenate([rows(tp, base), rows(t, base)], axis=1)
                return [(pltpu.roll(e, w * DIL, 1) if w else e)[:, 128:] for w in range(WIN)]

            lg = None
            for d in range(DH):
                q = rows(t, d)
                pr = [q * kk for kk in shifted(M + d)]
                lg = pr if lg is None else [a + b for a, b in zip(lg, pr)]
            lg = [l * (DH ** -0.5 * LOG2E) for l in lg]
            lg = [jnp.where(pos >= w * DIL, l, -1e9) if w else l for w, l in enumerate(lg)]
            m = lg[0]
            for l in lg[1:]:
                m = jnp.maximum(m, l)
            p = [jnp.exp2(l - m) for l in lg]
            den = p[0]
            for e in p[1:]:
                den = den + e
            inv = 1.0 / den
            p = [e * inv for e in p]
            for d in range(DH):
                o = None
                for pw, vv in zip(p, shifted(2 * M + d)):
                    o = pw * vv if o is None else o + pw * vv
                oa_s[u, pl.ds(d, H, stride=DH), :] = o
        oa = jnp.concatenate([oa_s[u] for u in range(CA // 128)], axis=1).astype(BF)
        a = jnp.dot(woat_s[...], oa, preferred_element_type=F32)
        b = jax.lax.dot_general(
            jnp.concatenate([wob[h] for h in range(H)], axis=1),
            jnp.concatenate([ctx_s[h, pl.ds(c0, CA), :] for h in range(H)], axis=1),
            NT, preferred_element_type=F32)
        g = jax.nn.sigmoid(jnp.concatenate(
            [qkv_s[i * (CA // 128) + u, 3 * M:3 * M + 1, :] for u in range(CA // 128)], axis=1))
        o_ref[:, pl.ds(c0, CA)] = (g * a + (1.0 - g) * b).astype(o_ref.dtype)
        return 0

    jax.lax.fori_loop(0, S // CA, p3, 0)


@jax.jit
def pallas_gated_mix__sliding_local_dilated__compressed_kv_cla__prompt_kernel(
    A_x, A_wqkv, A_wo, B_x, B_c_kv, B_w_q, B_w_uk, B_w_uv, B_w_o, gate_w,
):
    del B_x
    ins = (A_x.reshape(S, M).T, A_wqkv, A_wo, B_c_kv.reshape(S, DC),
           B_w_q.reshape(M * H, D), B_w_uk.reshape(DC * H, D), B_w_uv.reshape(DC * H, D),
           B_w_o.transpose(0, 2, 1))
    order = (0, 1, 2, 3, 4, 5, 6, 7)
    out = pl.pallas_call(
        _kernel,
        out_shape=jax.ShapeDtypeStruct((M, S), A_x.dtype),
        in_specs=[pl.BlockSpec(memory_space=pl.ANY)] * 8 + [pl.BlockSpec(memory_space=pltpu.VMEM)],
        scratch_shapes=[pltpu.VMEM(ins[i].shape, ins[i].dtype) for i in order] + [
            pltpu.VMEM((S, M), BF), pltpu.VMEM((NQ, M), BF), pltpu.VMEM((M, M), BF),
            pltpu.VMEM((S // 128, NQ, 128), F32), pltpu.VMEM((CA // 128, M, 128), F32),
            pltpu.VMEM((2, S, D), BF), pltpu.VMEM((2, S, D), BF), pltpu.VMEM((2, S, D), BF),
            pltpu.VMEM((H, S, D), BF),
            pltpu.VMEM((H, M, D), BF), pltpu.VMEM((H, DC, D), BF), pltpu.VMEM((H, DC, D), BF),
            pltpu.SemaphoreType.DMA((8,)),
        ],
        compiler_params=pltpu.CompilerParams(vmem_limit_bytes=110 * 1024 * 1024),
    )(*ins, gate_w.reshape(1, M))
    return out.T.reshape(1, S, M)
```

```python
import numpy as np
import jax
import jax.numpy as jnp
import jax.experimental.pallas as pl
import jax.experimental.pallas.tpu as pltpu

S = 2048
M = 576
H = 32
DH = 18
D = 128
DC = 512
WIN, DIL = 8, 2
BQ = 256
CA = 256
NQ = 3 * M + 16
LOG2E = 1.4426950408889634
BF = jnp.bfloat16
F32 = jnp.float32
NT = (((1,), (1,)), ((), ()))


def _split_heads(src, dst, i, kb):
    blk = src.bitcast(jnp.uint32).at[pl.ds(pl.multiple_of(i * (kb * H // 2), 8), kb * H // 2)]
    r0 = pl.multiple_of(i * kb, kb)
    for j in range(H // 2):
        w = blk[pl.ds(j, kb, stride=H // 2), :]
        dst[2 * j, pl.ds(r0, kb), :] = pltpu.bitcast(w << 16, F32).astype(BF)
        dst[2 * j + 1, pl.ds(r0, kb), :] = pltpu.bitcast(w & np.uint32(0xFFFF0000), F32).astype(BF)


def _pair(w_ref, j):
    return jnp.concatenate([w_ref[2 * j], w_ref[2 * j + 1]], axis=1)


def _kernel(xt_h, wqkv_h, woa_h, c_h, wq_h, wk_h, wv_h, wob_h, g_ref, o_ref,
            xt, wqkv, woa, c, wq, wk, wv, wob,
            x_s, wt_s, woat_s, qkv_s, oa_s, q_s, k_s, v_s, ctx_s, wq_s, wk_s, wv_s, sems):
    srcs = (wqkv_h, xt_h, c_h, wq_h, wk_h, wv_h, woa_h, wob_h)
    dsts = (wqkv, xt, c, wq, wk, wv, woa, wob)
    cps = [pltpu.make_async_copy(a, b, sems.at[i]) for i, (a, b) in enumerate(zip(srcs, dsts))]
    for cp in cps:
        cp.start()

    cps[0].wait()
    for t in range(3):
        wt_s[t * M:(t + 1) * M, :] = wqkv[:, t * M:(t + 1) * M].astype(F32).T.astype(BF)
    wt_s[3 * M:NQ, :] = jnp.broadcast_to(g_ref[...], (16, M))
    cps[1].wait()

    def p1(i, _):
        c0 = pl.multiple_of(i * CA, CA)
        xc = xt[:, pl.ds(c0, CA)]
        r = jnp.dot(wt_s[...], xc, preferred_element_type=F32)
        for u in range(CA // 128):
            qkv_s[i * (CA // 128) + u] = r[:, u * 128:(u + 1) * 128]
        x_s[pl.ds(c0, CA), :] = xc.astype(F32).T.astype(BF)
        return 0

    jax.lax.fori_loop(0, S // CA, p1, 0)

    for i in (2, 3, 4, 5):
        cps[i].wait()

    def split(i, _):
        _split_heads(wq, wq_s, i, M // 4)
        _split_heads(wk, wk_s, i, DC // 4)
        _split_heads(wv, wv_s, i, DC // 4)
        return 0

    jax.lax.fori_loop(0, 4, split, 0)
    tri = (jax.lax.broadcasted_iota(jnp.int32, (128, 128), 1)
           <= jax.lax.broadcasted_iota(jnp.int32, (128, 128), 0))
    NB = S // BQ

    def proj(h, slot, r0, r1):
        q = jnp.dot(x_s[r0:r1, :], wq_s[h], preferred_element_type=F32)
        q_s[slot, r0:r1, :] = (q * (D ** -0.5 * LOG2E)).astype(BF)
        kv = jnp.dot(c[r0:r1, :], jnp.concatenate([wk_s[h], wv_s[h]], axis=1),
                     preferred_element_type=F32).astype(BF)
        k_s[slot, r0:r1, :] = kv[:, :D]
        v_s[slot, r0:r1, :] = kv[:, D:]

    def scores(slot, i):
        r0, L = i * BQ, (i + 1) * BQ
        q = q_s[slot, r0:L, :]
        sf = jax.lax.dot_general(q, k_s[slot, 0:r0 + 128, :], NT, preferred_element_type=F32)
        sd = jax.lax.dot_general(q[128:], k_s[slot, r0 + 128:L, :], NT, preferred_element_type=F32)
        sd = jnp.where(tri, sd, -1e9)
        last = jnp.concatenate([jnp.where(tri, sf[:128, r0:], -1e9), sf[128:, r0:]], axis=0)
        sf = jnp.concatenate([sf[:, :r0], last], axis=1) if i else last
        cols = [sf[:, u:u + 128] for u in range(0, r0 + 128, 128)]
        m = cols[0]
        for t in cols[1:]:
            m = jnp.maximum(m, t)
        m = jnp.concatenate([m[:128], jnp.maximum(m[128:], sd)], axis=0)
        return sf, sd, jnp.max(m, axis=1, keepdims=True)

    def probs(sf, sd, m):
        pf = jnp.exp2(sf - m)
        pd = jnp.exp2(sd - m[128:])
        cols = [pf[:, u:u + 128] for u in range(0, pf.shape[1], 128)]
        l = cols[0]
        for t in cols[1:]:
            l = l + t
        l = jnp.concatenate([l[:128], l[128:] + pd], axis=0)
        return pf.astype(BF), pd.astype(BF), 1.0 / jnp.sum(l, axis=1, keepdims=True)

    def finish(h, slot, i, pf, pd, inv):
        r0, L = i * BQ, (i + 1) * BQ
        o = jnp.dot(pf, v_s[slot, 0:r0 + 128, :], preferred_element_type=F32)
        od = jnp.dot(pd, v_s[slot, r0 + 128:L, :], preferred_element_type=F32)
        o = jnp.concatenate([o[:128], o[128:] + od], axis=0)
        ctx_s[h, r0:L, :] = (o * inv).astype(BF)

    def head(h, hn, slot):
        st = scores(slot, 0)
        for i in range(NB):
            nxt = scores(slot, i + 1) if i + 1 < NB else None
            pr = probs(*st)
            proj(hn, 1 - slot, i * BQ, (i + 1) * BQ)
            finish(h, slot, i, *pr)
            st = nxt

    proj(0, 0, 0, S)

    def b_body(j, _):
        head(2 * j, 2 * j + 1, 0)
        head(2 * j + 1, jnp.minimum(2 * j + 2, H - 1), 1)
        return 0

    jax.lax.fori_loop(0, H // 2, b_body, 0)

    cps[6].wait()
    woat_s[...] = woa[...].astype(F32).T.astype(BF)
    cps[7].wait()

    def p3(i, _):
        c0 = pl.multiple_of(i * CA, CA)
        for u in range(CA // 128):
            t = i * (CA // 128) + u
            tp = jnp.maximum(t - 1, 0)
            lane = jax.lax.broadcasted_iota(jnp.int32, (H, 128), 1)
            pos = t * 128 + lane

            def rows(tt, base):
                return qkv_s[tt, pl.ds(base, H, stride=DH), :]

            def shifted(base):
                pv, cu = rows(tp, base), rows(t, base)
                return [pltpu.roll(jnp.where(lane >= 128 - w * DIL, pv, cu), w * DIL, 1) if w else cu
                        for w in range(WIN)]

            lg = None
            for d in range(DH):
                q = rows(t, d)
                pr = [q * kk for kk in shifted(M + d)]
                lg = pr if lg is None else [a + b for a, b in zip(lg, pr)]
            lg = [l * (DH ** -0.5 * LOG2E) for l in lg]
            lg = [jnp.where(pos >= w * DIL, l, -1e9) if w else l for w, l in enumerate(lg)]
            m = lg[0]
            for l in lg[1:]:
                m = jnp.maximum(m, l)
            p = [jnp.exp2(l - m) for l in lg]
            den = p[0]
            for e in p[1:]:
                den = den + e
            inv = 1.0 / den
            p = [e * inv for e in p]
            for d in range(DH):
                o = None
                for pw, vv in zip(p, shifted(2 * M + d)):
                    o = pw * vv if o is None else o + pw * vv
                oa_s[u, pl.ds(d, H, stride=DH), :] = o
        oa = jnp.concatenate([oa_s[u] for u in range(CA // 128)], axis=1).astype(BF)
        a = jnp.dot(woat_s[...], oa, preferred_element_type=F32)
        b = jax.lax.dot_general(
            jnp.concatenate([wob[h] for h in range(H)], axis=1),
            jnp.concatenate([ctx_s[h, pl.ds(c0, CA), :] for h in range(H)], axis=1),
            NT, preferred_element_type=F32)
        g = jax.nn.sigmoid(jnp.concatenate(
            [qkv_s[i * (CA // 128) + u, 3 * M:3 * M + 1, :] for u in range(CA // 128)], axis=1))
        o_ref[:, pl.ds(c0, CA)] = (g * a + (1.0 - g) * b).astype(o_ref.dtype)
        return 0

    jax.lax.fori_loop(0, S // CA, p3, 0)


@jax.jit
def pallas_gated_mix__sliding_local_dilated__compressed_kv_cla__prompt_kernel(
    A_x, A_wqkv, A_wo, B_x, B_c_kv, B_w_q, B_w_uk, B_w_uv, B_w_o, gate_w,
):
    del B_x
    ins = (A_x.reshape(S, M).T, A_wqkv, A_wo, B_c_kv.reshape(S, DC),
           B_w_q.reshape(M * H, D), B_w_uk.reshape(DC * H, D), B_w_uv.reshape(DC * H, D),
           B_w_o.transpose(0, 2, 1))
    order = (0, 1, 2, 3, 4, 5, 6, 7)
    out = pl.pallas_call(
        _kernel,
        out_shape=jax.ShapeDtypeStruct((M, S), A_x.dtype),
        in_specs=[pl.BlockSpec(memory_space=pl.ANY)] * 8 + [pl.BlockSpec(memory_space=pltpu.VMEM)],
        scratch_shapes=[pltpu.VMEM(ins[i].shape, ins[i].dtype) for i in order] + [
            pltpu.VMEM((S, M), BF), pltpu.VMEM((NQ, M), BF), pltpu.VMEM((M, M), BF),
            pltpu.VMEM((S // 128, NQ, 128), F32), pltpu.VMEM((CA // 128, M, 128), F32),
            pltpu.VMEM((2, S, D), BF), pltpu.VMEM((2, S, D), BF), pltpu.VMEM((2, S, D), BF),
            pltpu.VMEM((H, S, D), BF),
            pltpu.VMEM((H, M, D), BF), pltpu.VMEM((H, DC, D), BF), pltpu.VMEM((H, DC, D), BF),
            pltpu.SemaphoreType.DMA((8,)),
        ],
        compiler_params=pltpu.CompilerParams(vmem_limit_bytes=110 * 1024 * 1024),
    )(*ins, gate_w.reshape(1, M))
    return out.T.reshape(1, S, M)
```

```python
import numpy as np
import jax
import jax.numpy as jnp
import jax.experimental.pallas as pl
import jax.experimental.pallas.tpu as pltpu

S = 2048
M = 576
H = 32
DH = 18
D = 128
DC = 512
WIN, DIL = 8, 2
BQ = 256
CA = 256
HG = H * 128 // (4 * CA)
NQ = 3 * M + 16
LOG2E = 1.4426950408889634
BF = jnp.bfloat16
F32 = jnp.float32
NT = (((1,), (1,)), ((), ()))


def _split_heads(src, dst, i, kb):
    blk = src.bitcast(jnp.uint32).at[pl.ds(pl.multiple_of(i * (kb * H // 2), 8), kb * H // 2)]
    r0 = pl.multiple_of(i * kb, kb)
    for j in range(H // 2):
        w = blk[pl.ds(j, kb, stride=H // 2), :]
        dst[2 * j, pl.ds(r0, kb), :] = pltpu.bitcast(w << 16, F32).astype(BF)
        dst[2 * j + 1, pl.ds(r0, kb), :] = pltpu.bitcast(w & np.uint32(0xFFFF0000), F32).astype(BF)


def _pair(w_ref, j):
    return jnp.concatenate([w_ref[2 * j], w_ref[2 * j + 1]], axis=1)


def _kernel(xt_h, wqkv_h, woa_h, c_h, wq_h, wk_h, wv_h, wob_h, g_ref, o_ref,
            xt, wqkv, woa, c, wq, wk, wv, wob,
            x_s, wt_s, woat_s, qkv_s, oa_s, q_s, k_s, v_s, ctx_s, wq_s, wk_s, wv_s, sems):
    srcs = (wqkv_h, xt_h, c_h, wq_h, wk_h, wv_h, woa_h, wob_h)
    dsts = (wqkv, xt, c, wq, wk, wv, woa, wob)
    cps = [pltpu.make_async_copy(a, b, sems.at[i]) for i, (a, b) in enumerate(zip(srcs, dsts))]
    for cp in cps:
        cp.start()

    cps[0].wait()
    for t in range(3):
        wt_s[t * M:(t + 1) * M, :] = wqkv[:, t * M:(t + 1) * M].astype(F32).T.astype(BF)
    wt_s[3 * M:NQ, :] = jnp.broadcast_to(g_ref[...], (16, M))
    cps[1].wait()

    def p1(i, _):
        c0 = pl.multiple_of(i * CA, CA)
        xc = xt[:, pl.ds(c0, CA)]
        r = jnp.dot(wt_s[...], xc, preferred_element_type=F32)
        for u in range(CA // 128):
            qkv_s[i * (CA // 128) + u] = r[:, u * 128:(u + 1) * 128]
        x_s[pl.ds(c0, CA), :] = xc.astype(F32).T.astype(BF)
        return 0

    jax.lax.fori_loop(0, S // CA, p1, 0)

    for i in (2, 3, 4, 5):
        cps[i].wait()

    def split(i, _):
        _split_heads(wq, wq_s, i, M // 4)
        _split_heads(wk, wk_s, i, DC // 4)
        _split_heads(wv, wv_s, i, DC // 4)
        return 0

    jax.lax.fori_loop(0, 4, split, 0)
    tri = (jax.lax.broadcasted_iota(jnp.int32, (128, 128), 1)
           <= jax.lax.broadcasted_iota(jnp.int32, (128, 128), 0))
    NB = S // BQ

    def proj(h, slot, r0, r1):
        q = jnp.dot(x_s[r0:r1, :], wq_s[h], preferred_element_type=F32)
        q_s[slot, r0:r1, :] = (q * (D ** -0.5 * LOG2E)).astype(BF)
        kv = jnp.dot(c[r0:r1, :], jnp.concatenate([wk_s[h], wv_s[h]], axis=1),
                     preferred_element_type=F32).astype(BF)
        k_s[slot, r0:r1, :] = kv[:, :D]
        v_s[slot, r0:r1, :] = kv[:, D:]

    def scores(slot, i):
        r0, L = i * BQ, (i + 1) * BQ
        q = q_s[slot, r0:L, :]
        sf = jax.lax.dot_general(q, k_s[slot, 0:r0 + 128, :], NT, preferred_element_type=F32)
        sd = jax.lax.dot_general(q[128:], k_s[slot, r0 + 128:L, :], NT, preferred_element_type=F32)
        sd = jnp.where(tri, sd, -1e9)
        last = jnp.concatenate([jnp.where(tri, sf[:128, r0:], -1e9), sf[128:, r0:]], axis=0)
        sf = jnp.concatenate([sf[:, :r0], last], axis=1) if i else last
        cols = [sf[:, u:u + 128] for u in range(0, r0 + 128, 128)]
        m = cols[0]
        for t in cols[1:]:
            m = jnp.maximum(m, t)
        m = jnp.concatenate([m[:128], jnp.maximum(m[128:], sd)], axis=0)
        return sf, sd, jnp.max(m, axis=1, keepdims=True)

    def probs(sf, sd, m):
        pf = jnp.exp2(sf - m)
        pd = jnp.exp2(sd - m[128:])
        cols = [pf[:, u:u + 128] for u in range(0, pf.shape[1], 128)]
        l = cols[0]
        for t in cols[1:]:
            l = l + t
        l = jnp.concatenate([l[:128], l[128:] + pd], axis=0)
        return pf.astype(BF), pd.astype(BF), 1.0 / jnp.sum(l, axis=1, keepdims=True)

    def finish(h, slot, i, pf, pd, inv):
        r0, L = i * BQ, (i + 1) * BQ
        o = jnp.dot(pf, v_s[slot, 0:r0 + 128, :], preferred_element_type=F32)
        od = jnp.dot(pd, v_s[slot, r0 + 128:L, :], preferred_element_type=F32)
        o = jnp.concatenate([o[:128], o[128:] + od], axis=0)
        ctx_s[h, r0:L, :] = (o * inv).astype(BF)

    def head(h, hn, slot):
        st = scores(slot, 0)
        for i in range(NB):
            nxt = scores(slot, i + 1) if i + 1 < NB else None
            pr = probs(*st)
            proj(hn, 1 - slot, i * BQ, (i + 1) * BQ)
            finish(h, slot, i, *pr)
            st = nxt

    proj(0, 0, 0, S)

    def b_body(j, _):
        head(2 * j, 2 * j + 1, 0)
        head(2 * j + 1, jnp.minimum(2 * j + 2, H - 1), 1)
        return 0

    jax.lax.fori_loop(0, H // 2, b_body, 0)

    cps[6].wait()
    woat_s[...] = woa[...].astype(F32).T.astype(BF)
    cps[7].wait()

    def p3(i, _):
        c0 = pl.multiple_of(i * CA, CA)
        acc = []

        def bstep():
            hs = range(len(acc) * HG, (len(acc) + 1) * HG)
            r = jax.lax.dot_general(
                jnp.concatenate([wob[h] for h in hs], axis=1),
                jnp.concatenate([ctx_s[h, pl.ds(c0, CA), :] for h in hs], axis=1),
                NT, preferred_element_type=F32)
            acc.append(acc[-1] + r if acc else r)

        for u in range(CA // 128):
            t = i * (CA // 128) + u
            tp = jnp.maximum(t - 1, 0)
            lane = jax.lax.broadcasted_iota(jnp.int32, (H, 128), 1)
            pos = t * 128 + lane

            def rows(tt, base):
                return qkv_s[tt, pl.ds(base, H, stride=DH), :]

            def shifted(base):
                pv, cu = rows(tp, base), rows(t, base)
                return [pltpu.roll(jnp.where(lane >= 128 - w * DIL, pv, cu), w * DIL, 1) if w else cu
                        for w in range(WIN)]

            lg = None
            for d in range(DH):
                if d % 9 == 0:
                    bstep()
                q = rows(t, d)
                pr = [q * kk for kk in shifted(M + d)]
                lg = pr if lg is None else [a + b for a, b in zip(lg, pr)]
            lg = [l * (DH ** -0.5 * LOG2E) for l in lg]
            lg = [jnp.where(pos >= w * DIL, l, -1e9) if w else l for w, l in enumerate(lg)]
            m = lg[0]
            for l in lg[1:]:
                m = jnp.maximum(m, l)
            p = [jnp.exp2(l - m) for l in lg]
            den = p[0]
            for e in p[1:]:
                den = den + e
            inv = 1.0 / den
            p = [e * inv for e in p]
            for d in range(DH):
                if d % 9 == 0:
                    bstep()
                o = None
                for pw, vv in zip(p, shifted(2 * M + d)):
                    o = pw * vv if o is None else o + pw * vv
                oa_s[u, pl.ds(d, H, stride=DH), :] = o
        oa = jnp.concatenate([oa_s[u] for u in range(CA // 128)], axis=1).astype(BF)
        a = jnp.dot(woat_s[...], oa, preferred_element_type=F32)
        b = acc[-1]
        g = jax.nn.sigmoid(jnp.concatenate(
            [qkv_s[i * (CA // 128) + u, 3 * M:3 * M + 1, :] for u in range(CA // 128)], axis=1))
        o_ref[:, pl.ds(c0, CA)] = (g * a + (1.0 - g) * b).astype(o_ref.dtype)
        return 0

    jax.lax.fori_loop(0, S // CA, p3, 0)


@jax.jit
def pallas_gated_mix__sliding_local_dilated__compressed_kv_cla__prompt_kernel(
    A_x, A_wqkv, A_wo, B_x, B_c_kv, B_w_q, B_w_uk, B_w_uv, B_w_o, gate_w,
):
    del B_x
    ins = (A_x.reshape(S, M).T, A_wqkv, A_wo, B_c_kv.reshape(S, DC),
           B_w_q.reshape(M * H, D), B_w_uk.reshape(DC * H, D), B_w_uv.reshape(DC * H, D),
           B_w_o.transpose(0, 2, 1))
    order = (0, 1, 2, 3, 4, 5, 6, 7)
    out = pl.pallas_call(
        _kernel,
        out_shape=jax.ShapeDtypeStruct((M, S), A_x.dtype),
        in_specs=[pl.BlockSpec(memory_space=pl.ANY)] * 8 + [pl.BlockSpec(memory_space=pltpu.VMEM)],
        scratch_shapes=[pltpu.VMEM(ins[i].shape, ins[i].dtype) for i in order] + [
            pltpu.VMEM((S, M), BF), pltpu.VMEM((NQ, M), BF), pltpu.VMEM((M, M), BF),
            pltpu.VMEM((S // 128, NQ, 128), F32), pltpu.VMEM((CA // 128, M, 128), F32),
            pltpu.VMEM((2, S, D), BF), pltpu.VMEM((2, S, D), BF), pltpu.VMEM((2, S, D), BF),
            pltpu.VMEM((H, S, D), BF),
            pltpu.VMEM((H, M, D), BF), pltpu.VMEM((H, DC, D), BF), pltpu.VMEM((H, DC, D), BF),
            pltpu.SemaphoreType.DMA((8,)),
        ],
        compiler_params=pltpu.CompilerParams(vmem_limit_bytes=110 * 1024 * 1024),
    )(*ins, gate_w.reshape(1, M))
    return out.T.reshape(1, S, M)
```

```python
import numpy as np
import jax
import jax.numpy as jnp
import jax.experimental.pallas as pl
import jax.experimental.pallas.tpu as pltpu

S = 2048
M = 576
H = 32
DH = 18
D = 128
DC = 512
WIN, DIL = 8, 2
BQ = 256
CA = 256
HG = H * 128 // (4 * CA)
ORDER = ((0, 1, 2, 3, 4, 5, 6, 7), (7, 6, 5, 4, 3, 2, 1, 0))
NQ = 3 * M + 16
LOG2E = 1.4426950408889634
BF = jnp.bfloat16
F32 = jnp.float32
NT = (((1,), (1,)), ((), ()))


def _split_heads(src, dst, i, kb):
    blk = src.bitcast(jnp.uint32).at[pl.ds(pl.multiple_of(i * (kb * H // 2), 8), kb * H // 2)]
    r0 = pl.multiple_of(i * kb, kb)
    for j in range(H // 2):
        w = blk[pl.ds(j, kb, stride=H // 2), :]
        dst[2 * j, pl.ds(r0, kb), :] = pltpu.bitcast(w << 16, F32).astype(BF)
        dst[2 * j + 1, pl.ds(r0, kb), :] = pltpu.bitcast(w & np.uint32(0xFFFF0000), F32).astype(BF)


def _pair(w_ref, j):
    return jnp.concatenate([w_ref[2 * j], w_ref[2 * j + 1]], axis=1)


def _kernel(xt_h, wqkv_h, woa_h, c_h, wq_h, wk_h, wv_h, wob_h, g_ref, o_ref,
            xt, wqkv, woa, c, wq, wk, wv, wob,
            x_s, wt_s, woat_s, qkv_s, oa_s, q_s, k_s, v_s, ctx_s, wq_s, wk_s, wv_s, sems):
    srcs = (wqkv_h, xt_h, c_h, wq_h, wk_h, wv_h, woa_h, wob_h)
    dsts = (wqkv, xt, c, wq, wk, wv, woa, wob)
    cps = [pltpu.make_async_copy(a, b, sems.at[i]) for i, (a, b) in enumerate(zip(srcs, dsts))]
    for cp in cps:
        cp.start()

    cps[0].wait()
    for t in range(3):
        wt_s[t * M:(t + 1) * M, :] = wqkv[:, t * M:(t + 1) * M].astype(F32).T.astype(BF)
    wt_s[3 * M:NQ, :] = jnp.broadcast_to(g_ref[...], (16, M))
    cps[1].wait()

    def p1(i, _):
        c0 = pl.multiple_of(i * CA, CA)
        xc = xt[:, pl.ds(c0, CA)]
        r = jnp.dot(wt_s[...], xc, preferred_element_type=F32)
        for u in range(CA // 128):
            qkv_s[i * (CA // 128) + u] = r[:, u * 128:(u + 1) * 128]
        x_s[pl.ds(c0, CA), :] = xc.astype(F32).T.astype(BF)
        return 0

    jax.lax.fori_loop(0, S // CA, p1, 0)

    for i in (2, 3, 4, 5):
        cps[i].wait()

    def split(i, _):
        _split_heads(wq, wq_s, i, M // 4)
        _split_heads(wk, wk_s, i, DC // 4)
        _split_heads(wv, wv_s, i, DC // 4)
        return 0

    jax.lax.fori_loop(0, 4, split, 0)
    tri = (jax.lax.broadcasted_iota(jnp.int32, (128, 128), 1)
           <= jax.lax.broadcasted_iota(jnp.int32, (128, 128), 0))
    NB = S // BQ

    def proj(h, slot, r0, r1):
        q = jnp.dot(x_s[r0:r1, :], wq_s[h], preferred_element_type=F32)
        q_s[slot, r0:r1, :] = (q * (D ** -0.5 * LOG2E)).astype(BF)
        kv = jnp.dot(c[r0:r1, :], jnp.concatenate([wk_s[h], wv_s[h]], axis=1),
                     preferred_element_type=F32).astype(BF)
        k_s[slot, r0:r1, :] = kv[:, :D]
        v_s[slot, r0:r1, :] = kv[:, D:]

    def scores(slot, i):
        r0, L = i * BQ, (i + 1) * BQ
        q = q_s[slot, r0:L, :]
        sf = jax.lax.dot_general(q, k_s[slot, 0:r0 + 128, :], NT, preferred_element_type=F32)
        sd = jax.lax.dot_general(q[128:], k_s[slot, r0 + 128:L, :], NT, preferred_element_type=F32)
        sd = jnp.where(tri, sd, -1e9)
        last = jnp.concatenate([jnp.where(tri, sf[:128, r0:], -1e9), sf[128:, r0:]], axis=0)
        sf = jnp.concatenate([sf[:, :r0], last], axis=1) if i else last
        cols = [sf[:, u:u + 128] for u in range(0, r0 + 128, 128)]
        m = cols[0]
        for t in cols[1:]:
            m = jnp.maximum(m, t)
        m = jnp.concatenate([m[:128], jnp.maximum(m[128:], sd)], axis=0)
        return sf, sd, jnp.max(m, axis=1, keepdims=True)

    def probs(sf, sd, m):
        pf = jnp.exp2(sf - m)
        pd = jnp.exp2(sd - m[128:])
        cols = [pf[:, u:u + 128] for u in range(0, pf.shape[1], 128)]
        l = cols[0]
        for t in cols[1:]:
            l = l + t
        l = jnp.concatenate([l[:128], l[128:] + pd], axis=0)
        return pf.astype(BF), pd.astype(BF), 1.0 / jnp.sum(l, axis=1, keepdims=True)

    def finish(h, slot, i, pf, pd, inv):
        r0, L = i * BQ, (i + 1) * BQ
        o = jnp.dot(pf, v_s[slot, 0:r0 + 128, :], preferred_element_type=F32)
        od = jnp.dot(pd, v_s[slot, r0 + 128:L, :], preferred_element_type=F32)
        o = jnp.concatenate([o[:128], o[128:] + od], axis=0)
        ctx_s[h, r0:L, :] = (o * inv).astype(BF)

    def head(h, hn, slot):
        seq = ORDER[slot]
        st = scores(slot, seq[0])
        for n, i in enumerate(seq):
            nxt = scores(slot, seq[n + 1]) if n + 1 < NB else None
            pr = probs(*st)
            proj(hn, 1 - slot, n * BQ, (n + 1) * BQ)
            finish(h, slot, i, *pr)
            st = nxt

    proj(0, 0, 0, S)

    def b_body(j, _):
        head(2 * j, 2 * j + 1, 0)
        head(2 * j + 1, jnp.minimum(2 * j + 2, H - 1), 1)
        return 0

    jax.lax.fori_loop(0, H // 2, b_body, 0)

    cps[6].wait()
    woat_s[...] = woa[...].astype(F32).T.astype(BF)
    cps[7].wait()

    def p3(i, _):
        c0 = pl.multiple_of(i * CA, CA)
        acc = []

        def bstep():
            hs = range(len(acc) * HG, (len(acc) + 1) * HG)
            r = jax.lax.dot_general(
                jnp.concatenate([wob[h] for h in hs], axis=1),
                jnp.concatenate([ctx_s[h, pl.ds(c0, CA), :] for h in hs], axis=1),
                NT, preferred_element_type=F32)
            acc.append(acc[-1] + r if acc else r)

        for u in range(CA // 128):
            t = i * (CA // 128) + u
            tp = jnp.maximum(t - 1, 0)
            lane = jax.lax.broadcasted_iota(jnp.int32, (H, 128), 1)
            pos = t * 128 + lane

            def rows(tt, base):
                return qkv_s[tt, pl.ds(base, H, stride=DH), :]

            def shifted(base):
                pv, cu = rows(tp, base), rows(t, base)
                return [pltpu.roll(jnp.where(lane >= 128 - w * DIL, pv, cu), w * DIL, 1) if w else cu
                        for w in range(WIN)]

            lg = None
            for d in range(DH):
                if d % 9 == 0:
                    bstep()
                q = rows(t, d)
                pr = [q * kk for kk in shifted(M + d)]
                lg = pr if lg is None else [a + b for a, b in zip(lg, pr)]
            lg = [l * (DH ** -0.5 * LOG2E) for l in lg]
            lg = [jnp.where(pos >= w * DIL, l, -1e9) if w else l for w, l in enumerate(lg)]
            m = lg[0]
            for l in lg[1:]:
                m = jnp.maximum(m, l)
            p = [jnp.exp2(l - m) for l in lg]
            den = p[0]
            for e in p[1:]:
                den = den + e
            inv = 1.0 / den
            p = [e * inv for e in p]
            for d in range(DH):
                if d % 9 == 0:
                    bstep()
                o = None
                for pw, vv in zip(p, shifted(2 * M + d)):
                    o = pw * vv if o is None else o + pw * vv
                oa_s[u, pl.ds(d, H, stride=DH), :] = o
        oa = jnp.concatenate([oa_s[u] for u in range(CA // 128)], axis=1).astype(BF)
        a = jnp.dot(woat_s[...], oa, preferred_element_type=F32)
        b = acc[-1]
        g = jax.nn.sigmoid(jnp.concatenate(
            [qkv_s[i * (CA // 128) + u, 3 * M:3 * M + 1, :] for u in range(CA // 128)], axis=1))
        o_ref[:, pl.ds(c0, CA)] = (g * a + (1.0 - g) * b).astype(o_ref.dtype)
        return 0

    jax.lax.fori_loop(0, S // CA, p3, 0)


@jax.jit
def pallas_gated_mix__sliding_local_dilated__compressed_kv_cla__prompt_kernel(
    A_x, A_wqkv, A_wo, B_x, B_c_kv, B_w_q, B_w_uk, B_w_uv, B_w_o, gate_w,
):
    del B_x
    ins = (A_x.reshape(S, M).T, A_wqkv, A_wo, B_c_kv.reshape(S, DC),
           B_w_q.reshape(M * H, D), B_w_uk.reshape(DC * H, D), B_w_uv.reshape(DC * H, D),
           B_w_o.transpose(0, 2, 1))
    order = (0, 1, 2, 3, 4, 5, 6, 7)
    out = pl.pallas_call(
        _kernel,
        out_shape=jax.ShapeDtypeStruct((M, S), A_x.dtype),
        in_specs=[pl.BlockSpec(memory_space=pl.ANY)] * 8 + [pl.BlockSpec(memory_space=pltpu.VMEM)],
        scratch_shapes=[pltpu.VMEM(ins[i].shape, ins[i].dtype) for i in order] + [
            pltpu.VMEM((S, M), BF), pltpu.VMEM((NQ, M), BF), pltpu.VMEM((M, M), BF),
            pltpu.VMEM((S // 128, NQ, 128), F32), pltpu.VMEM((CA // 128, M, 128), F32),
            pltpu.VMEM((2, S, D), BF), pltpu.VMEM((2, S, D), BF), pltpu.VMEM((2, S, D), BF),
            pltpu.VMEM((H, S, D), BF),
            pltpu.VMEM((H, M, D), BF), pltpu.VMEM((H, DC, D), BF), pltpu.VMEM((H, DC, D), BF),
            pltpu.SemaphoreType.DMA((8,)),
        ],
        compiler_params=pltpu.CompilerParams(vmem_limit_bytes=110 * 1024 * 1024),
    )(*ins, gate_w.reshape(1, M))
    return out.T.reshape(1, S, M)
```

```python
import numpy as np
import jax
import jax.numpy as jnp
import jax.experimental.pallas as pl
import jax.experimental.pallas.tpu as pltpu

S = 2048
M = 576
H = 32
DH = 18
D = 128
DC = 512
WIN, DIL = 8, 2
BQ = 256
CA = 256
HG = H * 128 // (4 * CA)
ORDER = ((0, 1, 2, 3, 4, 5, 6, 7), (7, 6, 5, 4, 3, 2, 1, 0))
NQ = 3 * M + 16
LOG2E = 1.4426950408889634
BF = jnp.bfloat16
F32 = jnp.float32
NT = (((1,), (1,)), ((), ()))


def _split_heads(src, dst, i, kb):
    blk = src.bitcast(jnp.uint32).at[pl.ds(pl.multiple_of(i * (kb * H // 2), 8), kb * H // 2)]
    r0 = pl.multiple_of(i * kb, kb)
    for j in range(H // 2):
        w = blk[pl.ds(j, kb, stride=H // 2), :]
        dst[2 * j, pl.ds(r0, kb), :] = pltpu.bitcast(w << 16, F32).astype(BF)
        dst[2 * j + 1, pl.ds(r0, kb), :] = pltpu.bitcast(w & np.uint32(0xFFFF0000), F32).astype(BF)


def _pair(w_ref, j):
    return jnp.concatenate([w_ref[2 * j], w_ref[2 * j + 1]], axis=1)


def _kernel(xt_h, wqkv_h, woa_h, c_h, wq_h, wk_h, wv_h, wob_h, g_ref, o_ref,
            xt, wqkv, woa, c, wq, wk, wv, wob,
            x_s, wt_s, woat_s, qkv_s, oa_s, q_s, k_s, v_s, ctx_s, wq_s, wk_s, wv_s, o_s, sems, xsems, wsems):
    def col_cp(src, dst, i, sem):
        cs = pl.ds(pl.multiple_of(i * CA, CA), CA)
        return pltpu.make_async_copy(src.at[:, cs], dst.at[:, cs], sem)

    def w_cps(i):
        return [pltpu.make_async_copy(a.at[pl.ds(i * (a.shape[0] // 4), a.shape[0] // 4)],
                                      b.at[pl.ds(i * (a.shape[0] // 4), a.shape[0] // 4)],
                                      wsems.at[3 * i + n])
                for n, (a, b) in enumerate(((wq_h, wq), (wk_h, wk), (wv_h, wv)))]

    cps = [pltpu.make_async_copy(a, b, sems.at[i]) for i, (a, b) in
           enumerate(((wqkv_h, wqkv), (c_h, c), (woa_h, woa), (wob_h, wob)))]
    cps[0].start()
    for i in range(S // CA):
        col_cp(xt_h, xt, i, xsems.at[i]).start()

    cps[0].wait()
    for i in range(4):
        for cp in w_cps(i):
            cp.start()
    cps[1].start()
    for t in range(3):
        wt_s[t * M:(t + 1) * M, :] = wqkv[:, t * M:(t + 1) * M].astype(F32).T.astype(BF)
    wt_s[3 * M:NQ, :] = jnp.broadcast_to(g_ref[...], (16, M))

    def p1(i, _, split=False):
        col_cp(xt_h, xt, i, xsems.at[i]).wait()
        if split:
            for cp in w_cps(i - 4):
                cp.wait()
            _split_heads(wq, wq_s, i - 4, M // 4)
            _split_heads(wk, wk_s, i - 4, DC // 4)
            _split_heads(wv, wv_s, i - 4, DC // 4)
        c0 = pl.multiple_of(i * CA, CA)
        xc = xt[:, pl.ds(c0, CA)]
        r = jnp.dot(wt_s[...], xc, preferred_element_type=F32)
        for u in range(CA // 128):
            qkv_s[i * (CA // 128) + u] = r[:, u * 128:(u + 1) * 128]
        x_s[pl.ds(c0, CA), :] = xc.astype(F32).T.astype(BF)
        return 0

    jax.lax.fori_loop(0, 4, p1, 0)
    jax.lax.fori_loop(4, 8, lambda i, c_: p1(i, c_, True), 0)

    cps[1].wait()
    cps[2].start()
    cps[3].start()
    tri = (jax.lax.broadcasted_iota(jnp.int32, (128, 128), 1)
           <= jax.lax.broadcasted_iota(jnp.int32, (128, 128), 0))
    NB = S // BQ

    def proj(h, slot, r0, r1):
        q = jnp.dot(x_s[r0:r1, :], wq_s[h], preferred_element_type=F32)
        q_s[slot, r0:r1, :] = (q * (D ** -0.5 * LOG2E)).astype(BF)
        kv = jnp.dot(c[r0:r1, :], jnp.concatenate([wk_s[h], wv_s[h]], axis=1),
                     preferred_element_type=F32).astype(BF)
        k_s[slot, r0:r1, :] = kv[:, :D]
        v_s[slot, r0:r1, :] = kv[:, D:]

    def scores(slot, i):
        r0, L = i * BQ, (i + 1) * BQ
        q = q_s[slot, r0:L, :]
        sf = jax.lax.dot_general(q, k_s[slot, 0:r0 + 128, :], NT, preferred_element_type=F32)
        sd = jax.lax.dot_general(q[128:], k_s[slot, r0 + 128:L, :], NT, preferred_element_type=F32)
        sd = jnp.where(tri, sd, -1e9)
        last = jnp.concatenate([jnp.where(tri, sf[:128, r0:], -1e9), sf[128:, r0:]], axis=0)
        sf = jnp.concatenate([sf[:, :r0], last], axis=1) if i else last
        cols = [sf[:, u:u + 128] for u in range(0, r0 + 128, 128)]
        m = cols[0]
        for t in cols[1:]:
            m = jnp.maximum(m, t)
        m = jnp.concatenate([m[:128], jnp.maximum(m[128:], sd)], axis=0)
        return sf, sd, jnp.max(m, axis=1, keepdims=True)

    def probs(sf, sd, m):
        pf = jnp.exp2(sf - m)
        pd = jnp.exp2(sd - m[128:])
        cols = [pf[:, u:u + 128] for u in range(0, pf.shape[1], 128)]
        l = cols[0]
        for t in cols[1:]:
            l = l + t
        l = jnp.concatenate([l[:128], l[128:] + pd], axis=0)
        l = jnp.sum(l, axis=1, keepdims=True)
        r = pl.reciprocal(l, approx=True)
        return pf.astype(BF), pd.astype(BF), r * (2.0 - l * r)

    def finish(h, slot, i, pf, pd, inv):
        r0, L = i * BQ, (i + 1) * BQ
        o = jnp.dot(pf, v_s[slot, 0:r0 + 128, :], preferred_element_type=F32)
        od = jnp.dot(pd, v_s[slot, r0 + 128:L, :], preferred_element_type=F32)
        o = jnp.concatenate([o[:128], o[128:] + od], axis=0)
        ctx_s[h, r0:L, :] = (o * inv).astype(BF)

    def head(h, hn, slot):
        seq = ORDER[slot]
        st = scores(slot, seq[0])
        for n, i in enumerate(seq):
            nxt = scores(slot, seq[n + 1]) if n + 1 < NB else None
            pr = probs(*st)
            proj(hn, 1 - slot, n * BQ, (n + 1) * BQ)
            finish(h, slot, i, *pr)
            st = nxt

    proj(0, 0, 0, S)

    def b_body(j, _):
        head(2 * j, 2 * j + 1, 0)
        head(2 * j + 1, jnp.minimum(2 * j + 2, H - 1), 1)
        return 0

    jax.lax.fori_loop(0, H // 2, b_body, 0)

    cps[2].wait()
    woat_s[...] = woa[...].astype(F32).T.astype(BF)
    cps[3].wait()

    def p3(i, _):
        c0 = pl.multiple_of(i * CA, CA)
        acc = []

        def bstep():
            hs = range(len(acc) * HG, (len(acc) + 1) * HG)
            r = jax.lax.dot_general(
                jnp.concatenate([wob[h] for h in hs], axis=1),
                jnp.concatenate([ctx_s[h, pl.ds(c0, CA), :] for h in hs], axis=1),
                NT, preferred_element_type=F32)
            acc.append(acc[-1] + r if acc else r)

        for u in range(CA // 128):
            t = i * (CA // 128) + u
            tp = jnp.maximum(t - 1, 0)
            lane = jax.lax.broadcasted_iota(jnp.int32, (H, 128), 1)
            pos = t * 128 + lane

            def rows(tt, base):
                return qkv_s[tt, pl.ds(base, H, stride=DH), :]

            def shifted(base):
                pv, cu = rows(tp, base), rows(t, base)
                return [pltpu.roll(jnp.where(lane >= 128 - w * DIL, pv, cu), w * DIL, 1) if w else cu
                        for w in range(WIN)]

            lg = None
            for d in range(DH):
                if d % 9 == 0:
                    bstep()
                q = rows(t, d)
                pr = [q * kk for kk in shifted(M + d)]
                lg = pr if lg is None else [a + b for a, b in zip(lg, pr)]
            lg = [l * (DH ** -0.5 * LOG2E) for l in lg]
            lg = [jnp.where(pos >= w * DIL, l, -1e9) if w else l for w, l in enumerate(lg)]
            m = lg[0]
            for l in lg[1:]:
                m = jnp.maximum(m, l)
            p = [jnp.exp2(l - m) for l in lg]
            den = p[0]
            for e in p[1:]:
                den = den + e
            inv = 1.0 / den
            p = [e * inv for e in p]
            for d in range(DH):
                if d % 9 == 0:
                    bstep()
                o = None
                for pw, vv in zip(p, shifted(2 * M + d)):
                    o = pw * vv if o is None else o + pw * vv
                oa_s[u, pl.ds(d, H, stride=DH), :] = o
        oa = jnp.concatenate([oa_s[u] for u in range(CA // 128)], axis=1).astype(BF)
        a = jnp.dot(woat_s[...], oa, preferred_element_type=F32)
        b = acc[-1]
        g = jax.nn.sigmoid(jnp.concatenate(
            [qkv_s[i * (CA // 128) + u, 3 * M:3 * M + 1, :] for u in range(CA // 128)], axis=1))
        o_s[:, pl.ds(c0, CA)] = (g * a + (1.0 - g) * b).astype(o_s.dtype)
        col_cp(o_s, o_ref, i, xsems.at[i]).start()
        return 0

    jax.lax.fori_loop(0, S // CA, p3, 0)
    for i in range(S // CA):
        col_cp(o_s, o_ref, i, xsems.at[i]).wait()


@jax.jit
def pallas_gated_mix__sliding_local_dilated__compressed_kv_cla__prompt_kernel(
    A_x, A_wqkv, A_wo, B_x, B_c_kv, B_w_q, B_w_uk, B_w_uv, B_w_o, gate_w,
):
    del B_x
    ins = (A_x.reshape(S, M).T, A_wqkv, A_wo, B_c_kv.reshape(S, DC),
           B_w_q.reshape(M * H, D), B_w_uk.reshape(DC * H, D), B_w_uv.reshape(DC * H, D),
           B_w_o.transpose(0, 2, 1))
    order = (0, 1, 2, 3, 4, 5, 6, 7)
    out = pl.pallas_call(
        _kernel,
        out_shape=jax.ShapeDtypeStruct((M, S), A_x.dtype),
        in_specs=[pl.BlockSpec(memory_space=pl.ANY)] * 8 + [pl.BlockSpec(memory_space=pltpu.VMEM)],
        out_specs=pl.BlockSpec(memory_space=pl.ANY),
        scratch_shapes=[pltpu.VMEM(ins[i].shape, ins[i].dtype) for i in order] + [
            pltpu.VMEM((S, M), BF), pltpu.VMEM((NQ, M), BF), pltpu.VMEM((M, M), BF),
            pltpu.VMEM((S // 128, NQ, 128), F32), pltpu.VMEM((CA // 128, M, 128), F32),
            pltpu.VMEM((2, S, D), BF), pltpu.VMEM((2, S, D), BF), pltpu.VMEM((2, S, D), BF),
            pltpu.VMEM((H, S, D), BF),
            pltpu.VMEM((H, M, D), BF), pltpu.VMEM((H, DC, D), BF), pltpu.VMEM((H, DC, D), BF),
            pltpu.VMEM((M, S), A_x.dtype),
            pltpu.SemaphoreType.DMA((4,)), pltpu.SemaphoreType.DMA((8,)), pltpu.SemaphoreType.DMA((12,)),
        ],
        compiler_params=pltpu.CompilerParams(vmem_limit_bytes=110 * 1024 * 1024),
    )(*ins, gate_w.reshape(1, M))
    return out.T.reshape(1, S, M)
```
